```python
import os as _os
_os.environ.setdefault("JAX_PLATFORMS", "cpu")
import jax
import jax.numpy as jnp

def _softmax(x, axis=-1):
    return jax.nn.softmax(x, axis=axis)
def _gelu(x):
    return jax.nn.gelu(x, approximate=True)
def _silu(x):
    return jax.nn.silu(x)
def _sigmoid(x):
    return jax.nn.sigmoid(x)
def _layernorm(x, axis=-1, eps=1e-5):
    m = jnp.mean(x, axis=axis, keepdims=True)
    v = jnp.var(x, axis=axis, keepdims=True)
    return (x - m) / jnp.sqrt(v + eps)
def _scatter_add(tgt, idx, src, axis=0):
    return tgt.at[idx].add(src)
def _segment_sum(src, seg, n):
    return jax.ops.segment_sum(src, seg, n)
class _Rng:
    def __init__(self, key):
        self._k = key
    def _next(self):
        self._k, sub = jax.random.split(self._k)
        return sub
    def normal(self, shape):
        return jax.random.normal(self._next(), shape, dtype=jnp.bfloat16)
    def randint(self, lo, hi, shape):
        return jax.random.randint(self._next(), shape, lo, hi, dtype=jnp.int32)
    def uniform(self, shape, lo=0.0, hi=1.0):
        return jax.random.uniform(self._next(), shape, jnp.bfloat16, lo, hi)
    def permutation(self, n):
        return jax.random.permutation(self._next(), n)


kernel_name = 'interleave_layers__spectral_gfnet__dense_activation_gelu__prompt'

def setup_inputs():
    _rng = _Rng(jax.random.key(int.from_bytes(__import__("os").urandom(4), "little")))
    _w = (lambda a: (lambda t: t.astype(jnp.bfloat16) if jnp.issubdtype(t.dtype, jnp.floating) else t)(jnp.asarray(a)))
    def _A_setup():
        B, S, D = 1, 2048, 640
        Df = D // 2 + 1
        return {
            "x": _w((lambda *s: _rng.normal(s) * 0.05)(B, S, D)),
            "w_r": _w((lambda *s: _rng.normal(s) * 0.2)(S, Df) * 0.02),
            "w_i": _w((lambda *s: _rng.normal(s) * 0.2)(S, Df) * 0.02),
        }
    _A_in = _A_setup()

    def _B_setup():
        B, S, D, F = 1, 2048, 640, 1728
        return {
            "x": _w((lambda *s: _rng.normal(s) * 0.05)(B, S, D)),
            "w1": _w((lambda *s: _rng.normal(s) * 0.1)(D, F) * (D ** -0.5)),
            "b1": _w((lambda *s: _rng.normal(s) * 0.1)(F) * 0.01),
            "w2": _w((lambda *s: _rng.normal(s) * 0.1)(F, D) * (F ** -0.5)),
            "b2": _w((lambda *s: _rng.normal(s) * 0.1)(D) * 0.01),
        }
    _B_in = _B_setup()

    return {
        "A_x": _A_in["x"],
        "A_w_r": _A_in["w_r"],
        "A_w_i": _A_in["w_i"],
        "B_x": _B_in["x"],
        "B_w1": _B_in["w1"],
        "B_b1": _B_in["b1"],
        "B_w2": _B_in["w2"],
        "B_b2": _B_in["b2"],
    }

def reference(A_x, A_w_r, A_w_i, B_x, B_w1, B_b1, B_w2, B_b2):
    def _A_ref(x, w_r, w_i):
        B, S, D = x.shape
        X = (lambda x, axes=(-2,-1): jnp.fft.rfft2(x.astype(jnp.float32), axes=axes))(x, axes=(-2, -1))
        W = w_r + 1j * w_i
        X = X * W
        y = (lambda x, s, axes=(-2,-1): jnp.fft.irfft2(x, s=s, axes=axes).astype(jnp.bfloat16))(X, (S, D), axes=(-2, -1))
        return y

    def _B_ref(x, w1, b1, w2, b2):
        h = jnp.einsum("bsd,df->bsf", x, w1) + b1
        h = _gelu(h)
        return jnp.einsum("bsf,fd->bsd", h, w2) + b2

    x = A_x
    x = x + _A_ref(_layernorm(x, axis=-1), A_w_r, A_w_i)
    x = x + _B_ref(_layernorm(x, axis=-1), B_w1, B_b1, B_w2, B_b2)
    x = x + _A_ref(_layernorm(x, axis=-1), A_w_r, A_w_i)
    x = x + _B_ref(_layernorm(x, axis=-1), B_w1, B_b1, B_w2, B_b2)
    return x
```

```python
import functools
import math

import jax
import jax.numpy as jnp
import numpy as np
import jax.experimental.pallas as pl
import jax.experimental.pallas.tpu as pltpu

S, D, F = 2048, 640, 1728
DF = D // 2 + 1
P = 384
S1, S2 = 16, 128
RB = 256
NRB = S // RB


def _consts():
    d = np.arange(D)[:, None]
    k = np.arange(DF)[None, :]
    fd = np.zeros((D, 2 * P), np.float64)
    fd[:, :DF] = np.cos(2 * np.pi * ((d * k) % D) / D)
    fd[:, P:P + DF] = -np.sin(2 * np.pi * ((d * k) % D) / D)
    ck = np.full(DF, 2.0)
    ck[0] = 1.0
    ck[-1] = 1.0
    fdi = np.zeros((2 * P, D), np.float64)
    fdi[:DF] = ck[:, None] * np.cos(2 * np.pi * ((k.T * d.T) % D) / D) / (S * D)
    fdi[P:P + DF] = -ck[:, None] * np.sin(2 * np.pi * ((k.T * d.T) % D) / D) / (S * D)
    k2 = np.arange(S2)[:, None]
    s2 = np.arange(S2)[None, :]
    gf = np.zeros((S1, 2 * S2, 2 * S2), np.float64)
    gi = np.zeros((S1, 2 * S2, 2 * S2), np.float64)
    for k1 in range(S1):
        ang = -2 * np.pi * (((s2 * k2 * S1) + s2 * k1) % S) / S
        gr, gim = np.cos(ang), np.sin(ang)
        gf[k1, :S2, :S2] = gr
        gf[k1, :S2, S2:] = -gim
        gf[k1, S2:, :S2] = gim
        gf[k1, S2:, S2:] = gr
        hr, hi = gr.T, -gim.T
        gi[k1, :S2, :S2] = hr
        gi[k1, :S2, S2:] = -hi
        gi[k1, S2:, :S2] = hi
        gi[k1, S2:, S2:] = hr
    bf = jnp.bfloat16
    return (jnp.asarray(fd, bf), jnp.asarray(fdi, bf), jnp.asarray(gf, bf), jnp.asarray(gi, bf))


def _cmul_const(re, im, n, k, sign):
    k = k % n
    if k == 0:
        return re, im
    if 4 * k == n:
        return (-im, re) if sign > 0 else (im, -re)
    if 2 * k == n:
        return -re, -im
    if 4 * k == 3 * n:
        return (im, -re) if sign > 0 else (-im, re)
    c = math.cos(2 * math.pi * k / n)
    s = sign * math.sin(2 * math.pi * k / n)
    return re * c - im * s, re * s + im * c


def _fft_list(xs, sign):
    n = len(xs)
    if n == 1:
        return xs
    ev = _fft_list(xs[0::2], sign)
    od = _fft_list(xs[1::2], sign)
    out = [None] * n
    for k in range(n // 2):
        tr, ti = _cmul_const(od[k][0], od[k][1], n, k, sign)
        out[k] = (ev[k][0] + tr, ev[k][1] + ti)
        out[k + n // 2] = (ev[k][0] - tr, ev[k][1] - ti)
    return out


def _ln(xf):
    m = jnp.mean(xf, axis=-1, keepdims=True)
    xc = xf - m
    v = jnp.mean(xc * xc, axis=-1, keepdims=True)
    return xc * jax.lax.rsqrt(v + 1e-5)


def _gelu(h):
    c = math.sqrt(2.0 / math.pi)
    return 0.5 * h * (1.0 + jnp.tanh(c * (h + 0.044715 * (h * h * h))))


def _kernel(x_ref, wr_ref, wi_ref, w1_ref, b1_ref, w2_ref, b2_ref,
            fd_ref, fdi_ref, gf_ref, gi_ref, o_ref, y_s, a_s, q_s):
    f32, bf16 = jnp.float32, jnp.bfloat16

    def fwd_d(rows, xf):
        n = _ln(xf).astype(bf16)
        y_s[rows, :] = jnp.dot(n, fd_ref[...], preferred_element_type=f32)

    def p1(i, _):
        rows = pl.ds(pl.multiple_of(i * RB, RB), RB)
        fwd_d(rows, x_ref[rows, :].astype(f32))
        return 0
    jax.lax.fori_loop(0, NRB, p1, 0)

    for layer in range(2):
        def p2(r, _):
            r0 = pl.multiple_of(r * 8, 8)
            for c in range(P // 128):
                xs = [(y_s[pl.ds(s1 * S2 + r0, 8), pl.ds(c * 128, 128)],
                       y_s[pl.ds(s1 * S2 + r0, 8), pl.ds(P + c * 128, 128)]) for s1 in range(S1)]
                out = _fft_list(xs, -1)
                for k1 in range(S1):
                    a_s[k1, pl.ds(r0, 8), pl.ds(c * 128, 128)] = out[k1][0]
                    a_s[k1, pl.ds(S2 + r0, 8), pl.ds(c * 128, 128)] = out[k1][1]
            return 0
        jax.lax.fori_loop(0, S2 // 8, p2, 0)

        def p3(k1, _):
            a = a_s[k1].astype(bf16)
            z = jnp.dot(gf_ref[k1], a, preferred_element_type=f32)
            zr, zi = z[:S2], z[S2:]
            wr = wr_ref[k1].astype(f32)
            wi = wi_ref[k1].astype(f32)
            pr = zr * wr - zi * wi
            pi = zr * wi + zi * wr
            p = jnp.concatenate([pr, pi], axis=0).astype(bf16)
            a_s[k1] = jnp.dot(gi_ref[k1], p, preferred_element_type=f32)
            return 0
        jax.lax.fori_loop(0, S1, p3, 0)

        def p4(r, _):
            r0 = pl.multiple_of(r * 8, 8)
            for c in range(P // 128):
                xs = [(a_s[k1, pl.ds(r0, 8), pl.ds(c * 128, 128)],
                       a_s[k1, pl.ds(S2 + r0, 8), pl.ds(c * 128, 128)]) for k1 in range(S1)]
                out = _fft_list(xs, +1)
                for s1 in range(S1):
                    q_s[pl.ds(s1 * S2 + r0, 8), pl.ds(c * 128, 128)] = out[s1][0]
                    q_s[pl.ds(s1 * S2 + r0, 8), pl.ds(P + c * 128, 128)] = out[s1][1]
            return 0
        jax.lax.fori_loop(0, S2 // 8, p4, 0)

        def p5(i, _):
            rows = pl.ds(pl.multiple_of(i * RB, RB), RB)
            src = x_ref if layer == 0 else o_ref
            x0 = src[rows, :].astype(f32)
            y = jnp.dot(q_s[rows, :].astype(bf16), fdi_ref[...], preferred_element_type=f32)
            x1 = (x0 + y.astype(bf16).astype(f32)).astype(bf16).astype(f32)
            n = _ln(x1).astype(bf16)
            h = jnp.dot(n, w1_ref[...], preferred_element_type=f32) + b1_ref[...].astype(f32)
            g = _gelu(h).astype(bf16)
            m = jnp.dot(g, w2_ref[...], preferred_element_type=f32) + b2_ref[...].astype(f32)
            x2 = (x1 + m.astype(bf16).astype(f32)).astype(bf16)
            o_ref[rows, :] = x2
            if layer == 0:
                fwd_d(rows, x2.astype(f32))
            return 0
        jax.lax.fori_loop(0, NRB, p5, 0)


@jax.jit
def pallas_interleave_layers__spectral_gfnet__dense_activation_gelu__prompt_kernel(
    A_x, A_w_r, A_w_i, B_x, B_w1, B_b1, B_w2, B_b2,
):
    fd, fdi, gf, gi = _consts()
    x = A_x.reshape(S, D)

    def perm_w(w):
        w = jnp.pad(w, ((0, 0), (0, P - DF)))
        return w.reshape(S2, S1, P).transpose(1, 0, 2)

    wr, wi = perm_w(A_w_r), perm_w(A_w_i)
    b1 = B_b1.reshape(1, F)
    b2 = B_b2.reshape(1, D)
    out = pl.pallas_call(
        _kernel,
        out_shape=jax.ShapeDtypeStruct((S, D), jnp.bfloat16),
        scratch_shapes=[
            pltpu.VMEM((S, 2 * P), jnp.float32),
            pltpu.VMEM((S1, 2 * S2, P), jnp.float32),
            pltpu.VMEM((S, 2 * P), jnp.float32),
        ],
        compiler_params=pltpu.CompilerParams(vmem_limit_bytes=100 * 1024 * 1024),
    )(x, wr, wi, B_w1, b1, B_w2, b2, fd, fdi, gf, gi)
    return out.reshape(1, S, D)
```

```python
import functools
import math

import jax
import jax.numpy as jnp
import numpy as np
import jax.experimental.pallas as pl
import jax.experimental.pallas.tpu as pltpu

S, D, F = 2048, 640, 1728
DF = D // 2 + 1
P = 384
S1, S2 = 16, 128
RB = 512
NRB = S // RB
C1, C2 = math.cos(2 * math.pi / 5), math.cos(4 * math.pi / 5)
SN1, SN2 = math.sin(2 * math.pi / 5), math.sin(4 * math.pi / 5)


def _cplx_block(cr, ci):
    return np.block([[cr, ci], [-ci, cr]])


def _consts():
    d2 = np.arange(128)[:, None]
    k2 = np.arange(128)[None, :]
    gd = np.zeros((3, 256, 256), np.float64)
    gdi = np.zeros((3, 256, 256), np.float64)
    sel = np.zeros((DF, P), np.float64)
    for k1 in range(3):
        ang = -2 * np.pi * ((d2 * k2 * 5 + d2 * k1) % D) / D
        g = _cplx_block(np.cos(ang), np.sin(ang))
        sc = (1.0 if k1 == 0 else 2.0) / (S * D)
        gin = _cplx_block(np.cos(ang).T, -np.sin(ang).T) * sc
        kd = k1 + 5 * np.arange(128)
        mir = kd > D // 2
        g[:, 128:][:, mir] *= -1.0
        gin[128:, :][mir, :] *= -1.0
        gd[k1] = g
        gdi[k1] = gin
        src_col = np.where(mir, D - kd, kd)
        sel[src_col, k1 * 128 + np.arange(128)] = 1.0
    k2 = np.arange(S2)[:, None]
    s2 = np.arange(S2)[None, :]
    gf = np.zeros((S1, 2 * S2, 2 * S2), np.float64)
    gi = np.zeros((S1, 2 * S2, 2 * S2), np.float64)
    for k1 in range(S1):
        ang = -2 * np.pi * (((s2 * k2 * S1) + s2 * k1) % S) / S
        gr, gim = np.cos(ang), np.sin(ang)
        gf[k1] = np.block([[gr, -gim], [gim, gr]])
        hr, hi = gr.T, -gim.T
        gi[k1] = np.block([[hr, -hi], [hi, hr]])
    bf = jnp.bfloat16
    return (jnp.asarray(gd, bf), jnp.asarray(gdi, bf), jnp.asarray(gf, bf), jnp.asarray(gi, bf), jnp.asarray(sel, bf))


def _cmul_const(re, im, n, k, sign):
    k = k % n
    if k == 0:
        return re, im
    if 4 * k == n:
        return (-im, re) if sign > 0 else (im, -re)
    if 2 * k == n:
        return -re, -im
    if 4 * k == 3 * n:
        return (im, -re) if sign > 0 else (-im, re)
    c = math.cos(2 * math.pi * k / n)
    s = sign * math.sin(2 * math.pi * k / n)
    return re * c - im * s, re * s + im * c


def _fft_list(xs, sign):
    n = len(xs)
    if n == 1:
        return xs
    ev = _fft_list(xs[0::2], sign)
    od = _fft_list(xs[1::2], sign)
    out = [None] * n
    for k in range(n // 2):
        tr, ti = _cmul_const(od[k][0], od[k][1], n, k, sign)
        out[k] = (ev[k][0] + tr, ev[k][1] + ti)
        out[k + n // 2] = (ev[k][0] - tr, ev[k][1] - ti)
    return out


def _ln(xf):
    m = jnp.mean(xf, axis=-1, keepdims=True)
    xc = xf - m
    v = jnp.mean(xc * xc, axis=-1, keepdims=True)
    return xc * jax.lax.rsqrt(v + 1e-5)


def _gelu(h):
    c = math.sqrt(2.0 / math.pi)
    return 0.5 * h * (1.0 + jnp.tanh(c * (h + 0.044715 * (h * h * h))))


def _kernel(x_hbm, wr_hbm, wi_hbm, w1_hbm, b1_hbm, w2_hbm, b2_hbm,
            gd_hbm, gdi_hbm, gf_hbm, gi_hbm, sel_hbm, out_hbm, o_ref, y_s, a_s, q_s, wr_s, wi_s,
            x_ref, wr_ref, wi_ref, w1_ref, b1_ref, w2_ref, b2_ref,
            gd_ref, gdi_ref, gf_ref, gi_ref, sel_ref, xsem, wsem, sem):
    f32, bf16 = jnp.float32, jnp.bfloat16

    def xcopy(i):
        rows = pl.ds(i * RB, RB)
        return pltpu.make_async_copy(x_hbm.at[rows], x_ref.at[rows], xsem.at[i])

    def wcopy(i, which):
        cols = pl.ds(i * RB, RB)
        s, d = ((wr_hbm, wr_ref), (wi_hbm, wi_ref))[which]
        return pltpu.make_async_copy(s.at[:, cols], d.at[:, cols], wsem.at[which, i])
    others = [(sel_hbm, sel_ref), (gd_hbm, gd_ref),
              (gf_hbm, gf_ref), (gi_hbm, gi_ref), (gdi_hbm, gdi_ref),
              (w1_hbm, w1_ref), (b1_hbm, b1_ref), (w2_hbm, w2_ref), (b2_hbm, b2_ref)]
    cps = [pltpu.make_async_copy(s, d, sem.at[j]) for j, (s, d) in enumerate(others)]
    cps[0].start()
    for i in range(NRB):
        wcopy(i, 0).start()
        wcopy(i, 1).start()

    def pw(i, _):
        rows = pl.ds(pl.multiple_of(i * RB, RB), RB)

        @pl.when(i == 1)
        def _():
            cps[1].start()
            for j in range(NRB):
                xcopy(j).start()

        @pl.when(i == NRB - 1)
        def _():
            cps[2].start()
            cps[3].start()
        pltpu.make_async_copy(wr_hbm.at[:, rows], wr_ref.at[:, rows], wsem.at[0, i]).wait()
        pltpu.make_async_copy(wi_hbm.at[:, rows], wi_ref.at[:, rows], wsem.at[1, i]).wait()
        tn = (((0,), (0,)), ((), ()))
        wr = jax.lax.dot_general(wr_ref[:, rows], sel_ref[...], tn, preferred_element_type=f32)
        wi = jax.lax.dot_general(wi_ref[:, rows], sel_ref[...], tn, preferred_element_type=f32)
        for c in range(3):
            wr_s[c, rows, :] = wr[:, c * 128:(c + 1) * 128]
            wi_s[c, rows, :] = wi[:, c * 128:(c + 1) * 128]
        return 0
    cps[0].wait()
    with jax.named_scope("pw"):
        jax.lax.fori_loop(0, NRB, pw, 0)

    def fwd_d(rows, xf):
        n = _ln(xf)
        a = [n[:, j * 128:(j + 1) * 128] for j in range(5)]
        s14, s23 = a[1] + a[4], a[2] + a[3]
        d14, d23 = a[1] - a[4], a[2] - a[3]
        t0 = (a[0] + s14 + s23).astype(bf16)
        t1 = jnp.concatenate([a[0] + C1 * s14 + C2 * s23, -(SN1 * d14 + SN2 * d23)], axis=1).astype(bf16)
        t2 = jnp.concatenate([a[0] + C2 * s14 + C1 * s23, SN1 * d23 - SN2 * d14], axis=1).astype(bf16)
        o0 = jnp.dot(t0, gd_ref[0, :128, :], preferred_element_type=f32)
        o1 = jnp.dot(t1, gd_ref[1], preferred_element_type=f32)
        o2 = jnp.dot(t2, gd_ref[2], preferred_element_type=f32)
        for k1, o in enumerate((o0, o1, o2)):
            y_s[rows, pl.ds(k1 * 128, 128)] = o[:, :128]
            y_s[rows, pl.ds(P + k1 * 128, 128)] = o[:, 128:]

    def inv_d(rows):
        u = []
        for k1 in range(3):
            qk = jnp.concatenate([q_s[rows, pl.ds(k1 * 128, 128)], q_s[rows, pl.ds(P + k1 * 128, 128)]],
                                 axis=1).astype(bf16)
            g = gdi_ref[k1] if k1 > 0 else gdi_ref[0, :, :128]
            u.append(jnp.dot(qk, g, preferred_element_type=f32))
        u0, u1r, u1i, u2r, u2i = u[0], u[1][:, :128], u[1][:, 128:], u[2][:, :128], u[2][:, 128:]
        e1 = u0 + C1 * u1r + C2 * u2r
        o1 = SN1 * u1i + SN2 * u2i
        e2 = u0 + C2 * u1r + C1 * u2r
        o2 = SN2 * u1i - SN1 * u2i
        return jnp.concatenate([u0 + u1r + u2r, e1 - o1, e2 - o2, e2 + o2, e1 + o1], axis=1)

    def p1(i, _):
        rows = pl.ds(pl.multiple_of(i * RB, RB), RB)
        pltpu.make_async_copy(x_hbm.at[rows], x_ref.at[rows], xsem.at[i]).wait()
        fwd_d(rows, x_ref[rows, :].astype(f32))
        return 0
    cps[1].wait()
    with jax.named_scope("p1"):
        jax.lax.fori_loop(0, NRB, p1, 0)

    for c in cps[4:]:
        c.start()
    for layer in range(2):
        def p2(r, _):
            r0 = pl.multiple_of(r * 8, 8)
            for c in range(P // 128):
                xs = [(y_s[pl.ds(s1 * S2 + r0, 8), pl.ds(c * 128, 128)],
                       y_s[pl.ds(s1 * S2 + r0, 8), pl.ds(P + c * 128, 128)]) for s1 in range(S1)]
                out = _fft_list(xs, -1)
                for k1 in range(S1):
                    a_s[k1, pl.ds(r0, 8), pl.ds(c * 128, 128)] = out[k1][0]
                    a_s[k1, pl.ds(S2 + r0, 8), pl.ds(c * 128, 128)] = out[k1][1]
            return 0
        with jax.named_scope("p2"):
            jax.lax.fori_loop(0, S2 // 8, p2, 0)

        if layer == 0:
            for c in cps[2:4]:
                c.wait()
        def p3(k1, _):
            a = a_s[k1].astype(bf16)
            z = jnp.dot(gf_ref[k1], a, preferred_element_type=f32)
            zr, zi = z[:S2], z[S2:]
            wr = jnp.concatenate([wr_s[c, pl.ds(k1, S2, stride=S1), :] for c in range(3)], axis=1)
            wi = jnp.concatenate([wi_s[c, pl.ds(k1, S2, stride=S1), :] for c in range(3)], axis=1)
            pr = zr * wr - zi * wi
            pi = zr * wi + zi * wr
            p = jnp.concatenate([pr, pi], axis=0).astype(bf16)
            a_s[k1] = jnp.dot(gi_ref[k1], p, preferred_element_type=f32)
            return 0
        with jax.named_scope("p3"):
            jax.lax.fori_loop(0, S1, p3, 0, unroll=4)

        def p4(r, _):
            r0 = pl.multiple_of(r * 8, 8)
            for c in range(P // 128):
                xs = [(a_s[k1, pl.ds(r0, 8), pl.ds(c * 128, 128)],
                       a_s[k1, pl.ds(S2 + r0, 8), pl.ds(c * 128, 128)]) for k1 in range(S1)]
                out = _fft_list(xs, +1)
                for s1 in range(S1):
                    q_s[pl.ds(s1 * S2 + r0, 8), pl.ds(c * 128, 128)] = out[s1][0]
                    q_s[pl.ds(s1 * S2 + r0, 8), pl.ds(P + c * 128, 128)] = out[s1][1]
            return 0
        with jax.named_scope("p4"):
            jax.lax.fori_loop(0, S2 // 8, p4, 0)

        if layer == 0:
            for c in cps[4:]:
                c.wait()
        def p5(i, _):
            rows = pl.ds(pl.multiple_of(i * RB, RB), RB)
            src = x_ref if layer == 0 else o_ref
            x0 = src[rows, :].astype(f32)
            y = inv_d(rows)
            x1 = (x0 + y.astype(bf16).astype(f32)).astype(bf16).astype(f32)
            n = _ln(x1).astype(bf16)
            h = jax.lax.dot_general(n, w1_ref[...], (((1,), (1,)), ((), ())), preferred_element_type=f32) + b1_ref[...].astype(f32)
            g = _gelu(h).astype(bf16)
            m = jnp.dot(g, w2_ref[...], preferred_element_type=f32) + b2_ref[...].astype(f32)
            x2 = (x1 + m.astype(bf16).astype(f32)).astype(bf16)
            o_ref[rows, :] = x2
            if layer == 1:
                pltpu.make_async_copy(o_ref.at[rows], out_hbm.at[rows], xsem.at[i]).start()
            if layer == 0:
                fwd_d(rows, x2.astype(f32))
            return 0
        with jax.named_scope("p5"):
            jax.lax.fori_loop(0, NRB, p5, 0)
    for i in range(NRB):
        rows = pl.ds(i * RB, RB)
        pltpu.make_async_copy(o_ref.at[rows], out_hbm.at[rows], xsem.at[i]).wait()


@jax.jit
def pallas_interleave_layers__spectral_gfnet__dense_activation_gelu__prompt_kernel(
    A_x, A_w_r, A_w_i, B_x, B_w1, B_b1, B_w2, B_b2,
):
    gd, gdi, gf, gi, sel = _consts()
    x = A_x.reshape(S, D)
    b1 = B_b1.reshape(1, F)
    b2 = B_b2.reshape(1, D)
    args = (x, A_w_r.T, A_w_i.T, B_w1.T, b1, B_w2, b2, gd, gdi, gf, gi, sel)
    out = pl.pallas_call(
        _kernel,
        out_shape=jax.ShapeDtypeStruct((S, D), jnp.bfloat16),
        out_specs=pl.BlockSpec(memory_space=pl.ANY),
        scratch_shapes=[
            pltpu.VMEM((S, D), jnp.bfloat16),
            pltpu.VMEM((S, 2 * P), jnp.float32),
            pltpu.VMEM((S1, 2 * S2, P), jnp.float32),
            pltpu.VMEM((S, 2 * P), jnp.float32),
            pltpu.VMEM((3, S, 128), jnp.float32),
            pltpu.VMEM((3, S, 128), jnp.float32),
        ] + [pltpu.VMEM(a.shape, a.dtype) for a in args] + [
            pltpu.SemaphoreType.DMA((NRB,)),
            pltpu.SemaphoreType.DMA((2, NRB)),
            pltpu.SemaphoreType.DMA((9,)),
        ],
        in_specs=[pl.BlockSpec(memory_space=pl.ANY)] * len(args),
        compiler_params=pltpu.CompilerParams(vmem_limit_bytes=100 * 1024 * 1024),
    )(*args)
    return out.reshape(1, S, D)
```

```python
import math

import jax
import jax.numpy as jnp
import numpy as np
import jax.experimental.pallas as pl
import jax.experimental.pallas.tpu as pltpu

S, D, F = 2048, 640, 1728
DF = D // 2 + 1
P = 384
S1, S2 = 16, 128
NG = 4
WC = 512
C1, C2 = math.cos(2 * math.pi / 5), math.cos(4 * math.pi / 5)
SN1, SN2 = math.sin(2 * math.pi / 5), math.sin(4 * math.pi / 5)


def _consts():
    d2 = np.arange(128)[:, None]
    k2 = np.arange(128)[None, :]
    gd = np.zeros((3, 256, 256), np.float64)
    gdi = np.zeros((3, 256, 256), np.float64)
    for k1 in range(3):
        ang = -2 * np.pi * ((d2 * k2 * 5 + d2 * k1) % D) / D
        cr, ci = np.cos(ang), np.sin(ang)
        g = np.block([[cr, ci], [-ci, cr]])
        sc = (1.0 if k1 == 0 else 2.0) / (S * D)
        gin = np.block([[cr.T, -ci.T], [ci.T, cr.T]]) * sc
        mir = (k1 + 5 * np.arange(128)) > D // 2
        g[:, 128:][:, mir] *= -1.0
        gin[128:, :][mir, :] *= -1.0
        gd[k1] = g
        gdi[k1] = gin
    k2 = np.arange(S2)[:, None]
    s2 = np.arange(S2)[None, :]
    gf = np.zeros((S1, 2 * S2, 2 * S2), np.float64)
    gi = np.zeros((S1, 2 * S2, 2 * S2), np.float64)
    for k1 in range(S1):
        ang = -2 * np.pi * (((s2 * k2 * S1) + s2 * k1) % S) / S
        gr, gim = np.cos(ang), np.sin(ang)
        gf[k1] = np.block([[gr, -gim], [gim, gr]])
        gi[k1] = np.block([[gr.T, gim.T], [-gim.T, gr.T]])
    bf = jnp.bfloat16
    return (jnp.asarray(gd, bf), jnp.asarray(gdi, bf), jnp.asarray(gf, bf), jnp.asarray(gi, bf))


def _ln(xf):
    m = jnp.mean(xf, axis=-1, keepdims=True)
    xc = xf - m
    v = jnp.mean(xc * xc, axis=-1, keepdims=True)
    return xc * jax.lax.rsqrt(v + 1e-5)


def _gelu(h):
    c = math.sqrt(2.0 / math.pi)
    return 0.5 * h * (1.0 + jnp.tanh(c * (h + 0.044715 * (h * h * h))))


def _rot(v, q):
    re, im = v
    q %= 4
    if q == 0:
        return re, im
    if q == 1:
        return -im, re
    if q == 2:
        return -re, -im
    return im, -re


def _radix4(v, sign):
    t0 = (v[0][0] + v[2][0], v[0][1] + v[2][1])
    t1 = (v[0][0] - v[2][0], v[0][1] - v[2][1])
    t2 = (v[1][0] + v[3][0], v[1][1] + v[3][1])
    t3 = _rot((v[1][0] - v[3][0], v[1][1] - v[3][1]), sign)
    return [(t0[0] + t2[0], t0[1] + t2[1]), (t1[0] + t3[0], t1[1] + t3[1]),
            (t0[0] - t2[0], t0[1] - t2[1]), (t1[0] - t3[0], t1[1] - t3[1])]


def _kernel(x_hbm, wr_hbm, wi_hbm, w1_hbm, b1_hbm, w2_hbm, b2_hbm,
            gd_hbm, gdi_hbm, gf_hbm, gi_hbm, out_hbm,
            o_ref, b_s, e_s, wr_s, wi_s,
            x_ref, wr_ref, wi_ref, w1_ref, b1_ref, w2_ref, b2_ref,
            gd_ref, gdi_ref, gf_ref, gi_ref, sel_ref, osem, wsem, sem):
    f32, bf16 = jnp.float32, jnp.bfloat16
    NW = S // WC

    def wcopy(i, which):
        cols = pl.ds(i * WC, WC)
        s, d = ((wr_hbm, wr_ref), (wi_hbm, wi_ref))[which]
        return pltpu.make_async_copy(s.at[:, cols], d.at[:, cols], wsem.at[which, i])
    pairs = [(x_hbm, x_ref), (gd_hbm, gd_ref), (gf_hbm, gf_ref), (gi_hbm, gi_ref), (gdi_hbm, gdi_ref),
             (w1_hbm, w1_ref), (b1_hbm, b1_ref), (w2_hbm, w2_ref), (b2_hbm, b2_ref)]

    def cp(j):
        return pltpu.make_async_copy(pairs[j][0], pairs[j][1], sem.at[j])
    for i in range(NW):
        wcopy(i, 0).start()
        wcopy(i, 1).start()
    srow = jax.lax.broadcasted_iota(jnp.int32, (DF, P), 0)
    scol = jax.lax.broadcasted_iota(jnp.int32, (DF, P), 1)
    kd = (scol >> 7) + 5 * (scol & 127)
    kd = jnp.where(kd > D // 2, D - kd, kd)
    sel_ref[...] = jnp.where(srow == kd, 1.0, 0.0).astype(bf16)

    def pw(i, _):
        rows = pl.ds(pl.multiple_of(i * WC, WC), WC)

        @pl.when(i == 1)
        def _():
            cp(0).start()
            cp(1).start()

        @pl.when(i == NW - 1)
        def _():
            cp(2).start()
            cp(3).start()
        pltpu.make_async_copy(wr_hbm.at[:, rows], wr_ref.at[:, rows], wsem.at[0, i]).wait()
        pltpu.make_async_copy(wi_hbm.at[:, rows], wi_ref.at[:, rows], wsem.at[1, i]).wait()
        tn = (((0,), (0,)), ((), ()))
        wr = jax.lax.dot_general(wr_ref[:, rows], sel_ref[...], tn, preferred_element_type=f32)
        wi = jax.lax.dot_general(wi_ref[:, rows], sel_ref[...], tn, preferred_element_type=f32)
        for c in range(3):
            wr_s[c, rows, :] = wr[:, c * 128:(c + 1) * 128]
            wi_s[c, rows, :] = wi[:, c * 128:(c + 1) * 128]
        return 0
    with jax.named_scope("pw"):
        jax.lax.fori_loop(0, NW, pw, 0)

    def slab(i, j):
        return pl.ds(pl.multiple_of((i + NG * j) * S2, S2), S2)

    def twiddles(i, sign):
        out = []
        for kq in range(1, 4):
            ang = jnp.full((1, 128), sign * 2 * math.pi * kq / 16, f32) * i.astype(f32)
            out.append((jnp.cos(ang), jnp.sin(ang)))
        return out

    def fwd_d(i, xf):
        n = _ln(xf)
        a = [n[:, j * 128:(j + 1) * 128] for j in range(5)]
        s14, s23 = a[1] + a[4], a[2] + a[3]
        d14, d23 = a[1] - a[4], a[2] - a[3]
        t0 = (a[0] + s14 + s23).astype(bf16)
        t1 = jnp.concatenate([a[0] + C1 * s14 + C2 * s23, -(SN1 * d14 + SN2 * d23)], axis=1).astype(bf16)
        t2 = jnp.concatenate([a[0] + C2 * s14 + C1 * s23, SN1 * d23 - SN2 * d14], axis=1).astype(bf16)
        os_ = (jnp.dot(t0, gd_ref[0, :128, :], preferred_element_type=f32),
               jnp.dot(t1, gd_ref[1], preferred_element_type=f32),
               jnp.dot(t2, gd_ref[2], preferred_element_type=f32))
        tw = twiddles(i, -1)
        for k1, o in enumerate(os_):
            v = [(o[j * S2:(j + 1) * S2, :128], o[j * S2:(j + 1) * S2, 128:]) for j in range(4)]
            b = _radix4(v, -1)
            for kq in range(4):
                re, im = b[kq]
                if kq:
                    c, s = tw[kq - 1]
                    re, im = re * c - im * s, re * s + im * c
                b_s[i, kq, pl.ds(0, S2), pl.ds(k1 * 128, 128)] = re
                b_s[i, kq, pl.ds(S2, S2), pl.ds(k1 * 128, 128)] = im

    def inv_d(i):
        tw = twiddles(i, +1)
        u = []
        for k1 in range(3):
            v = []
            for kq in range(4):
                re = e_s[i, kq, pl.ds(0, S2), pl.ds(k1 * 128, 128)]
                im = e_s[i, kq, pl.ds(S2, S2), pl.ds(k1 * 128, 128)]
                if kq:
                    c, s = tw[kq - 1]
                    re, im = re * c - im * s, re * s + im * c
                v.append((re, im))
            y = _radix4(v, +1)
            qk = jnp.concatenate([jnp.concatenate([y[j][0], y[j][1]], axis=1) for j in range(4)],
                                 axis=0).astype(bf16)
            g = gdi_ref[k1] if k1 > 0 else gdi_ref[0, :, :128]
            u.append(jnp.dot(qk, g, preferred_element_type=f32))
        u0, u1r, u1i, u2r, u2i = u[0], u[1][:, :128], u[1][:, 128:], u[2][:, :128], u[2][:, 128:]
        e1 = u0 + C1 * u1r + C2 * u2r
        o1 = SN1 * u1i + SN2 * u2i
        e2 = u0 + C2 * u1r + C1 * u2r
        o2 = SN2 * u1i - SN1 * u2i
        return jnp.concatenate([u0 + u1r + u2r, e1 - o1, e2 - o2, e2 + o2, e1 + o1], axis=1)

    def gather(ref, i):
        return jnp.concatenate([ref[slab(i, j), :] for j in range(4)], axis=0)

    def p1(i, _):
        fwd_d(i, gather(x_ref, i).astype(f32))
        return 0
    cp(0).wait()
    cp(1).wait()
    with jax.named_scope("p1"):
        jax.lax.fori_loop(0, NG, p1, 0)
    for j in range(4, len(pairs)):
        cp(j).start()

    for layer in range(2):
        if layer == 0:
            cp(2).wait()
            cp(3).wait()

        with jax.named_scope("p3"):
            for kp in range(4):
                def p3(kq, _):
                    k1 = kq + 4 * kp
                    parts = []
                    for i in range(4):
                        blk = b_s[i, kq]
                        parts.append(_rot((blk[:S2], blk[S2:]), -i * kp))
                    ar = (parts[0][0] + parts[1][0]) + (parts[2][0] + parts[3][0])
                    ai = (parts[0][1] + parts[1][1]) + (parts[2][1] + parts[3][1])
                    a = jnp.concatenate([ar, ai], axis=0).astype(bf16)
                    z = jnp.dot(gf_ref[k1], a, preferred_element_type=f32)
                    zr, zi = z[:S2], z[S2:]
                    wr = jnp.concatenate([wr_s[c, pl.ds(k1, S2, stride=S1), :] for c in range(3)], axis=1)
                    wi = jnp.concatenate([wi_s[c, pl.ds(k1, S2, stride=S1), :] for c in range(3)], axis=1)
                    pr = zr * wr - zi * wi
                    pi = zr * wi + zi * wr
                    p = jnp.concatenate([pr, pi], axis=0).astype(bf16)
                    cc = jnp.dot(gi_ref[k1], p, preferred_element_type=f32)
                    for i in range(4):
                        re, im = _rot((cc[:S2], cc[S2:]), i * kp)
                        if kp == 0:
                            e_s[i, kq, pl.ds(0, S2), :] = re
                            e_s[i, kq, pl.ds(S2, S2), :] = im
                        else:
                            e_s[i, kq, pl.ds(0, S2), :] += re
                            e_s[i, kq, pl.ds(S2, S2), :] += im
                    return 0
                jax.lax.fori_loop(0, 4, p3, 0, unroll=True)

        if layer == 0:
            for j in range(4, len(pairs)):
                cp(j).wait()

        def p5(i, _):
            x0 = gather(x_ref if layer == 0 else o_ref, i).astype(f32)
            y = inv_d(i)
            x1 = (x0 + y.astype(bf16).astype(f32)).astype(bf16).astype(f32)
            n = _ln(x1).astype(bf16)
            h = (jax.lax.dot_general(n, w1_ref[...], (((1,), (1,)), ((), ())), preferred_element_type=f32)
                 + b1_ref[...].astype(f32).reshape(1, F))
            g = _gelu(h).astype(bf16)
            m = jnp.dot(g, w2_ref[...], preferred_element_type=f32) + b2_ref[...].astype(f32).reshape(1, D)
            x2 = (x1 + m.astype(bf16).astype(f32)).astype(bf16)
            for j in range(4):
                o_ref[slab(i, j), :] = x2[j * S2:(j + 1) * S2]
                if layer == 1:
                    pltpu.make_async_copy(o_ref.at[slab(i, j)], out_hbm.at[slab(i, j)],
                                          osem.at[i + NG * j]).start()
            if layer == 0:
                fwd_d(i, x2.astype(f32))
            return 0
        with jax.named_scope("p5"):
            jax.lax.fori_loop(0, NG, p5, 0)

    for t in range(S1):
        rows = pl.ds(t * S2, S2)
        pltpu.make_async_copy(o_ref.at[rows], out_hbm.at[rows], osem.at[t]).wait()


@jax.jit
def pallas_interleave_layers__spectral_gfnet__dense_activation_gelu__prompt_kernel(
    A_x, A_w_r, A_w_i, B_x, B_w1, B_b1, B_w2, B_b2,
):
    gd, gdi, gf, gi = _consts()
    x = A_x.reshape(S, D)
    args = (x, A_w_r.T, A_w_i.T, B_w1.T, B_b1, B_w2, B_b2, gd, gdi, gf, gi)
    out = pl.pallas_call(
        _kernel,
        out_shape=jax.ShapeDtypeStruct((S, D), jnp.bfloat16),
        in_specs=[pl.BlockSpec(memory_space=pl.ANY)] * len(args),
        out_specs=pl.BlockSpec(memory_space=pl.ANY),
        scratch_shapes=[
            pltpu.VMEM((S, D), jnp.bfloat16),
            pltpu.VMEM((NG, 4, 2 * S2, P), jnp.float32),
            pltpu.VMEM((NG, 4, 2 * S2, P), jnp.float32),
            pltpu.VMEM((3, S, 128), jnp.float32),
            pltpu.VMEM((3, S, 128), jnp.float32),
        ] + [pltpu.VMEM(a.shape, a.dtype) for a in args] + [
            pltpu.VMEM((DF, P), jnp.bfloat16),
            pltpu.SemaphoreType.DMA((S1,)),
            pltpu.SemaphoreType.DMA((2, S // WC)),
            pltpu.SemaphoreType.DMA((9,)),
        ],
        compiler_params=pltpu.CompilerParams(vmem_limit_bytes=100 * 1024 * 1024),
    )(*args)
    return out.reshape(1, S, D)
```
